```python
import os as _os
_os.environ.setdefault("JAX_PLATFORMS", "cpu")
import jax
import jax.numpy as jnp

def _softmax(x, axis=-1):
    return jax.nn.softmax(x, axis=axis)
def _gelu(x):
    return jax.nn.gelu(x, approximate=True)
def _silu(x):
    return jax.nn.silu(x)
def _sigmoid(x):
    return jax.nn.sigmoid(x)
def _layernorm(x, axis=-1, eps=1e-5):
    m = jnp.mean(x, axis=axis, keepdims=True)
    v = jnp.var(x, axis=axis, keepdims=True)
    return (x - m) / jnp.sqrt(v + eps)
def _scatter_add(tgt, idx, src, axis=0):
    return tgt.at[idx].add(src)
def _segment_sum(src, seg, n):
    return jax.ops.segment_sum(src, seg, n)
class _Rng:
    def __init__(self, key):
        self._k = key
    def _next(self):
        self._k, sub = jax.random.split(self._k)
        return sub
    def normal(self, shape):
        return jax.random.normal(self._next(), shape, dtype=jnp.bfloat16)
    def randint(self, lo, hi, shape):
        return jax.random.randint(self._next(), shape, lo, hi, dtype=jnp.int32)
    def uniform(self, shape, lo=0.0, hi=1.0):
        return jax.random.uniform(self._next(), shape, jnp.bfloat16, lo, hi)
    def permutation(self, n):
        return jax.random.permutation(self._next(), n)


kernel_name = 'sequential_preLN__softmax_full_mha__dense_activation_squared_relu__prompt'

def setup_inputs():
    _rng = _Rng(jax.random.key(int.from_bytes(__import__("os").urandom(4), "little")))
    _w = (lambda a: (lambda t: t.astype(jnp.bfloat16) if jnp.issubdtype(t.dtype, jnp.floating) else t)(jnp.asarray(a)))
    def _A_setup():
        B, S, D = 1, 2048, 448
        return {
            "x": _w((lambda *s: _rng.normal(s) * 0.05)(B, S, D)),
            "wqkv": _w((lambda *s: _rng.normal(s) * 0.05)(D, 3 * D)),
            "wo": _w((lambda *s: _rng.normal(s) * 0.05)(D, D)),
        }
    _A_in = _A_setup()

    def _B_setup():
        B, S, D, F = 1, 2048, 448, 1792
        return {
            "x": _w((lambda *s: _rng.normal(s) * 0.05)(B, S, D)),
            "w1": _w((lambda *s: _rng.normal(s) * 0.05)(D, F)),
            "b1": _w((lambda *s: _rng.normal(s) * 0.05)(F)),
            "w2": _w((lambda *s: _rng.normal(s) * 0.05)(F, D)),
            "b2": _w((lambda *s: _rng.normal(s) * 0.05)(D)),
        }
    _B_in = _B_setup()

    return {
        "A_x": _A_in["x"],
        "A_wqkv": _A_in["wqkv"],
        "A_wo": _A_in["wo"],
        "B_x": _B_in["x"],
        "B_w1": _B_in["w1"],
        "B_b1": _B_in["b1"],
        "B_w2": _B_in["w2"],
        "B_b2": _B_in["b2"],
    }

def reference(A_x, A_wqkv, A_wo, B_x, B_w1, B_b1, B_w2, B_b2):
    def _A_ref(x, wqkv, wo):
        B, S, D = x.shape
        H = 16; Dh = D // H
        qkv = (lambda x, *d: x.transpose(*d))((x @ wqkv).reshape(B, S, 3, H, Dh), 2, 0, 3, 1, 4)
        q, k, v = qkv[0], qkv[1], qkv[2]
        scale = Dh ** -0.5
        scores = jnp.einsum("bhqd,bhkd->bhqk", q, k) * scale
        p = _softmax(scores, axis=-1)
        o = jnp.einsum("bhqk,bhkd->bhqd", p, v)
        return (lambda x, *d: x.transpose(*d))(o, 0, 2, 1, 3).reshape(B, S, D) @ wo

    def _B_ref(x, w1, b1, w2, b2):
        h = jnp.einsum("bsd,df->bsf", x, w1) + b1
        zero = jnp.zeros_like(h)
        r = jnp.where(h > zero, h, zero)
        h = r * r
        out = jnp.einsum("bsf,fd->bsd", h, w2) + b2
        return out

    x = A_x
    h = x + _A_ref(_layernorm(x, axis=-1), A_wqkv, A_wo)
    h2 = h + _B_ref(_layernorm(h, axis=-1), B_w1, B_b1, B_w2, B_b2)
    return h2
```

```python
import functools
import math

import jax
import jax.numpy as jnp
from jax import lax
import jax.experimental.pallas as pl
import jax.experimental.pallas.tpu as pltpu

S, D, H, DH, F = 2048, 448, 16, 28, 1792
TB = 512
NB = S // TB
KC = 128
NC = S // KC
G = 4 * DH
HP = 32
EPS = 1e-5
QSCALE = DH ** -0.5 * math.log2(math.e)
BF = jnp.bfloat16
F32 = jnp.float32


def _dot(a, b):
  return jnp.dot(a, b, preferred_element_type=F32)


def _layernorm_cols(x):
  mu = jnp.sum(x, axis=0, keepdims=True) * (1.0 / D)
  xc = x - mu
  var = jnp.sum(xc * xc, axis=0, keepdims=True) * (1.0 / D)
  return xc * lax.rsqrt(var + EPS)


def _head_window(h):
  return DH * h - 4 * (h % 2)


def make_kernel(UN=4, LAG=1):
  NU = NB * H

  def kern(x_hbm, wqkv_hbm, wo_hbm, w1_hbm, b1_hbm, w2t_hbm, b2_hbm, out_hbm,
           x_v, wqkv_v, wo_v, w1_v, b1_v, w2t_v, b2_v,
           wqkvt, wot, w1t, b2c, q_s, k_s, v_s, o_s, sa, sb, h_s, hn_s, out_v,
           in_sem, out_sem):
    x_cp = [pltpu.make_async_copy(x_hbm.at[:, pl.ds(i * TB, TB)], x_v.at[i], in_sem.at[i])
            for i in range(NB)]
    wqkv_cp = pltpu.make_async_copy(wqkv_hbm, wqkv_v, in_sem.at[NB])
    rest_cp = [pltpu.make_async_copy(a, b, in_sem.at[NB + 1 + i]) for i, (a, b) in enumerate(
        [(wo_hbm, wo_v), (w1_hbm, w1_v), (b1_hbm, b1_v), (w2t_hbm, w2t_v), (b2_hbm, b2_v)])]
    x_cp[0].start()
    wqkv_cp.start()
    for c in x_cp[1:]:
      c.start()
    for c in rest_cp:
      c.start()

    x_cp[0].wait()
    wqkv_cp.wait()
    wqkvt[...] = wqkv_v[...].T
    sub = lax.broadcasted_iota(jnp.int32, (HP, TB), 0)

    def qkv_block(i):
      xn = _layernorm_cols(x_v[i].astype(F32)).astype(BF)
      kt = _dot(wqkvt[D:2 * D, :], xn)
      for g in range(4):
        kg = jnp.concatenate([kt[g * G:(g + 1) * G], jnp.zeros((128 - G, TB), F32)], axis=0)
        k_s[g, i * TB:(i + 1) * TB, :] = kg.astype(BF).T
      vt = _dot(wqkvt[2 * D:3 * D, :], xn)
      for h in range(H):
        lo = _head_window(h)
        own = (sub >= 4) if h % 2 else (sub < DH)
        v_s[h, :, i * TB:(i + 1) * TB] = jnp.where(own, vt[lo:lo + HP], 1.0).astype(BF)
      qt = _dot(wqkvt[0:D, :], xn)
      q_s[i] = (qt * QSCALE).astype(BF)

    qkv_block(0)
    for c in x_cp[1:]:
      c.wait()
    for i in range(1, NB):
      qkv_block(i)

    row = lax.broadcasted_iota(jnp.int32, (G, TB), 0)

    def load_q(qb, g, j):
      q = q_s[qb, pl.ds(pl.multiple_of(g * G, 16), G), :]
      keep = (row >= j * DH) & (row < (j + 1) * DH)
      return jnp.where(keep, q.astype(F32), 0.0).astype(BF)

    def qk(qm, g, buf, c, m8):
      s = _dot(k_s[g, c * KC:(c + 1) * KC, :G], qm)
      buf[c * KC:(c + 1) * KC, :] = s
      mm = jnp.max(s.reshape(KC // 8, 8, TB), axis=0)
      return mm if m8 is None else jnp.maximum(m8, mm)

    def pv(h, buf, c, m, acc, z):
      s = buf[pl.ds(pl.multiple_of(z + c * KC, KC), KC), :]
      p = jnp.exp2(s - m).astype(BF)
      r = _dot(v_s[h, :, c * KC:(c + 1) * KC], p)
      return r if acc is None else acc + r

    def finish(qb, h, odd, acc):
      l = acc[0:1] if odd else acc[HP - 1:HP]
      o_s[qb, pl.ds(pl.multiple_of(h * HP, HP), HP), :] = (acc * (1.0 / l)).astype(BF)

    bufs = (sa, sb)

    def step(u0, k, m8, z, last=False, filler=None):
      u = u0 + k
      m = jnp.max(m8, axis=0, keepdims=True)
      if not last:
        gn = (u0 // 4 + (k + 1) // 4)
        qm = load_q(gn // 4, gn % 4, (k + 1) % 4)
      m8, acc = None, None
      for c in range(NC + LAG):
        if c < NC and not last:
          m8 = qk(qm, gn % 4, bufs[(k + 1) % 2], c, m8)
        if filler is not None:
          filler(c)
        if c >= LAG:
          acc = pv(u % H, bufs[k % 2], c - LAG, m, acc, z)
      finish(u // H, u % H, k % 2 == 1, acc)
      return m8

    qm = load_q(0, 0, 0)
    m8 = None
    for c in range(NC):
      m8 = qk(qm, 0, sa, c, m8)

    def body(it, carry):
      m8, _ = carry
      z = (it // NU) * KC
      for k in range(UN):
        m8 = step(it * UN, k, m8, z)
      return m8, z

    m8, z = lax.fori_loop(0, NU // UN - 1, body, (m8, jnp.int32(0)))

    for c in rest_cp:
      c.wait()
    subo = lax.broadcasted_iota(jnp.int32, (HP, D), 0)
    for g in range(4):
      wo32 = wo_v[g * G:(g + 1) * G, :].astype(F32)
      rows = []
      for j in range(4):
        lo = _head_window(j)
        own = (subo >= 4) if j % 2 else (subo < DH)
        rows.append(jnp.where(own, wo32[lo:lo + HP], 0.0))
      wot[:, g * 128:(g + 1) * 128] = jnp.concatenate(rows, axis=0).astype(BF).T
    w1t[:, 0:384] = w1_v[0:384, :].T
    b1 = b1_v[...].astype(F32).reshape(1, F)
    tail = jnp.where(lax.broadcasted_iota(jnp.int32, (64, F), 0) == 0, b1, 0.0).astype(BF)
    w1t[:, 384:512] = jnp.concatenate([w1_v[384:D, :], tail], axis=0).T
    b2c[...] = jnp.broadcast_to(b2_v[...].astype(F32).reshape(1, D), (128, D)).T

    def proj_ln(i):
      h = x_v[i].astype(F32) + _dot(wot[...], o_s[i])
      h_s[i] = h
      hn_s[i, 0:D, :] = _layernorm_cols(h).astype(BF)
      hn_s[i, D:512, :] = jnp.ones((512 - D, TB), BF)

    for k in range(UN - 1):
      m8 = step(NU - UN, k, m8, z)
    step(NU - UN, UN - 1, m8, z, last=True, filler=lambda c: proj_ln(0) if c == 0 else None)

    def out_cp(i):
      return pltpu.make_async_copy(out_v.at[i], out_hbm.at[:, pl.ds(i * TB, TB)], out_sem.at[i])

    def ffn(i):
      a = jnp.maximum(_dot(w1t[...], hn_s[i]), 0.0)
      a = (a * a).astype(BF)
      f = _dot(w2t_v[...], a)
      out_v[i] = (h_s[i] + jnp.tile(b2c[...], (1, TB // 128)) + f).astype(BF)

    def body3(i, _):
      ffn(i)
      proj_ln(i + 1)
      out_cp(i).start()

    lax.fori_loop(0, NB - 1, body3, None)
    ffn(NB - 1)
    out_cp(NB - 1).start()
    for i in range(NB):
      out_cp(i).wait()

  return kern


def build(name="fused", flags=None, **kw):
  kern = make_kernel(**kw)

  def f(A_x, A_wqkv, A_wo, B_x, B_w1, B_b1, B_w2, B_b2):
    del B_x
    hbm = pl.BlockSpec(memory_space=pltpu.HBM)
    out_t = pl.pallas_call(
        kern,
        out_shape=jax.ShapeDtypeStruct((D, S), BF),
        in_specs=[hbm] * 7,
        out_specs=hbm,
        scratch_shapes=[
            pltpu.VMEM((NB, D, TB), BF),
            pltpu.VMEM((D, 3 * D), BF),
            pltpu.VMEM((D, D), BF),
            pltpu.VMEM((D, F), BF),
            pltpu.VMEM((F,), BF),
            pltpu.VMEM((D, F), BF),
            pltpu.VMEM((D,), BF),
            pltpu.VMEM((3 * D, D), BF),
            pltpu.VMEM((D, 512), BF),
            pltpu.VMEM((F, 512), BF),
            pltpu.VMEM((D, 128), F32),
            pltpu.VMEM((NB, D, TB), BF),
            pltpu.VMEM((4, S, 128), BF),
            pltpu.VMEM((H, HP, S), BF),
            pltpu.VMEM((NB, H * HP, TB), BF),
            pltpu.VMEM((S, TB), F32),
            pltpu.VMEM((S, TB), F32),
            pltpu.VMEM((NB, D, TB), F32),
            pltpu.VMEM((NB, 512, TB), BF),
            pltpu.VMEM((NB, D, TB), BF),
            pltpu.SemaphoreType.DMA((NB + 6,)),
            pltpu.SemaphoreType.DMA((NB,)),
        ],
        compiler_params=pltpu.CompilerParams(vmem_limit_bytes=100 << 20, flags=flags),
        name=name,
    )(A_x.reshape(S, D).T, A_wqkv, A_wo, B_w1, B_b1, B_w2.T, B_b2)
    return out_t.T.reshape(1, S, D)

  return jax.jit(f)


pallas_sequential_preLN__softmax_full_mha__dense_activation_squared_relu__prompt_kernel = build()
```

```python
import functools
import math

import jax
import jax.numpy as jnp
from jax import lax
import jax.experimental.pallas as pl
import jax.experimental.pallas.tpu as pltpu

S, D, H, DH, F = 2048, 448, 16, 28, 1792
TB = 256
NB = S // TB
KC = 256
NC = S // KC
G = 4 * DH
HP = 32
NV = 192
VPU_KEYS = (192, 192, 192, 192, 192, 160, 192, 160)
LAG = 2
KEY_SHIFT = (3, 3, 3, 2, 3, 5, 8, 6, 6)
VALUE_SHIFT = (3, 4)
EPS = 1e-5
QSCALE = DH ** -0.5 * math.log2(math.e)
BF, F32, I32 = jnp.bfloat16, jnp.float32, jnp.int32


def _dot(a, b):
  return lax.dot_general(a, b, (((1,), (0,)), ((), ())), preferred_element_type=F32)


def _pack(x):
  return pltpu.bitcast(x.astype(BF), I32)


def _unpack(x):
  return pltpu.bitcast(x, BF)


def _at(start, size, align):
  return pl.ds(start if isinstance(start, int) else pl.multiple_of(start, align), size)


def _fold(x):
  return functools.reduce(jnp.add, [x[i:i + 8] for i in range(0, x.shape[0], 8)])


def _chain(*tasks):
  for task in tasks:
    yield from task


def _take(task, n):
  for _, piece in zip(range(n), task):
    yield piece


def _run(task):
  for _ in task:
    pass


def _window(h):
  return DH * h - (HP - DH) * (h % 2)


def _store_cyclic(dst, w, odd):
  if odd:
    dst[4:36, :] = w
    dst[0:8, :] = w[24:32]
  else:
    dst[0:32, :] = w
    dst[28:36, :] = w[0:8]


def _strassen_lhs(w11, w12, w21, w22):
  return [w11 + w22, w21 + w22, w11, w22, w11 + w12, w21 - w11, w12 - w22]


def _strassen_rhs(a1, a2, b1, b2):
  return [a1 - b2, a1, b1 - b2, a2 - a1, b2, b1 - a1, a2 - b2]


def _key_cuts(first):
  sizes = [(S - first) // 32 // NC] * NC
  for j in range((S - first) // 32 % NC):
    sizes[(2 * j + 2 * j // NC) % NC] += 1
  cuts = [first]
  for n in sizes:
    cuts += [cuts[-1] + 16 * n, cuts[-1] + 32 * n]
  return cuts


class _Pacer:
  def __init__(self, zero):
    self.never = lax.broadcasted_iota(I32, (8, 128), 0) < zero
    self.tasks, self.passes, self.results = [], 0, []

  def add(self, task, pieces, slots, lead=0, ramp=0):
    self.tasks.append(dict(task=task, pieces=pieces, slots=slots, slot=0, issued=-lead, ramp=ramp))

  def tie(self, vreg, shift=None):
    for t in self.tasks:
      t["slot"] += 1
      goal = t["pieces"] * t["slot"] // t["slots"] + (shift or 0) - max(0, t["ramp"] - t["slot"])
      values = [next(t["task"], []) for _ in range(t["issued"], goal)]
      t["issued"] = max(t["issued"], goal)
      if shift is not None:
        values = [v(t["slot"]) if callable(v) else v for v in values[-1:]]
        shift = 0
      for x in sum(values, []):
        x = x[0:8, 0:128]
        vreg = lax.select(self.never, x if x.dtype == vreg.dtype else pltpu.bitcast(x, vreg.dtype), vreg)
    return vreg

  def dot(self, lhs, rhs):
    step = 8 if lhs.dtype == I32 else 16
    tiles = []
    for c in range(0, lhs.shape[1], 128):
      tile = lhs[:, c:c + 128]
      if self.tasks and self.passes % 4 == 0:
        tile = jnp.concatenate([tile[i:i + 8] if i % step else self.tie(tile[i:i + 8])
                                for i in range(0, tile.shape[0], 8)], axis=0)
      self.passes += 1
      tiles.append(tile)
    lhs = jnp.concatenate(tiles, axis=1)
    return _dot(_unpack(lhs) if lhs.dtype == I32 else lhs, rhs)

  def mark(self, x):
    self.results.append((self.passes, x))
    return x

  def anchor(self, x, back=16):
    old = [r for n, r in self.results if n <= self.passes - back]
    if not old:
      return x
    return jnp.concatenate([lax.select(self.never, old[-1][0:8, 0:128], x[i:i + 8])
                            for i in range(0, x.shape[0], 8)], axis=0)

  def finish(self):
    for t in self.tasks:
      _run(t["task"])
    self.tasks = []


def _block_kernel(x_hbm, wqkv_hbm, wo_hbm, w1_hbm, b1_hbm, w2t_hbm, b2_hbm, out_hbm,
                  x_v, wqkv_v, wo_v, w1_v, w2t_v, wqkv_t, wo_t, w1_t, wqkv_s, wo_s, w1_s, w2_s, b1_c, b2_c,
                  q_s, k_s, v_s, o_s, h_s, out_v, qc_s, kc_s, skew_s, kb0, kb1, acc_s, e0, e1, e2,
                  act_s, rest_s, h0_s, s0, s1, s2, s3, b1_v, b2_v, in_sem, out_sem, zero_s):
  scores = (s0, s1, s2, s3)
  cols = lambda p: _at(p * TB, TB, TB)

  xs = lambda lo, hi: (x_hbm.at[:, lo * TB:hi * TB], x_v.at[:, lo * TB:hi * TB])
  ws = lambda lo, hi: (wqkv_hbm.at[:, lo:hi], wqkv_v.at[:, lo:hi])
  stages = [[ws(0, 256)], [xs(0, 1)], [xs(1, 2)], [ws(256, 512)], [ws(896, 3 * D)], [ws(512, 896), xs(2, 3)],
            [xs(3, NB)], [(wo_hbm, wo_v), (b1_hbm, b1_v), (b2_hbm, b2_v), (w2t_hbm, w2t_v), (w1_hbm, w1_v)]]
  stages = [[pltpu.make_async_copy(src, dst, in_sem.at[i]) for src, dst in stage]
            for i, stage in enumerate(stages)]
  for copy in sum(stages, []):
    copy.start()

  def wait(i):
    for copy in stages[i]:
      copy.wait()

  @pl.loop(0, NB)
  def _(i):
    zero_s[i] = 0

  zs = [zero_s[i] for i in range(NB)]
  z0 = zs[0]

  def encode(load, dst, via_memory=False):
    def put(i, r, x):
      dst[i, r:r + 16, :] = x
      return [x[8:]]

    for r in range(0, 128, 16):
      x1, x2 = load(r), load(128 + r)
      e = [put(i, r, x) for i, x in enumerate(_strassen_rhs(x1[:, :128], x2[:, :128], x1[:, 128:], x2[:, 128:]))]
      yield from ([], [], [dst[z0 + 6, r:r + 8, :]]) if via_memory else (e[0], e[2] + e[5], e[3] + e[6])
    for r in range(0, 64, 16):
      u, v, w = load(256 + r), load(320 + r), load(384 + r)
      au, bv = u[:, :128].astype(BF).astype(F32), v[:, 128:].astype(BF).astype(F32)
      halves = ((au, bv), (v[:, :128] - bv, w[:, :128]), (u[:, 128:] - au, w[:, 128:]))
      e = [put(7 + i, r, lo) + put(7 + i, 64 + r, hi) for i, (lo, hi) in enumerate(halves)]
      yield from ([], [], [dst[z0 + 9, r:r + 8, :]]) if via_memory else e

  def layernorm(load, dst, via_memory=False):
    for r in range(0, D, 32):
      part = _fold(load(_at(zs[1] + r, 32, 16)))
      acc = acc + part if r else part
      yield [acc, acc[:, 128:]]
    mean = jnp.sum(acc, axis=0, keepdims=True) * (1.0 / D)
    for r in range(0, D, 32):
      centred = load(_at(zs[2] + r, 32, 16)) - mean
      part = _fold(centred * centred)
      acc = acc + part if r else part
      yield [acc, acc[:, 128:]]
    rstd = lax.rsqrt(jnp.sum(acc, axis=0, keepdims=True) * (1.0 / D) + EPS)
    yield from encode(lambda r: (load(_at(zs[3] + r, 16, 16)) - mean) * rstd, dst, via_memory)

  def transpose_tiles(dst, src, *spans):
    u, v, w = 256, 320, 384
    for t, parts in ((0, [(0, 128)]), (1, [(128, 128)]), (2, [(u, 128)]), (4, [(u, 64), (w, 64)]), (3, [(v, 128)])):
      for c, n in spans:
        dst[t, c // 2:(c + n) // 2, :] = _pack(jnp.concatenate([src[r:r + k, c:c + n] for r, k in parts], axis=0).T)

  def tile_sums(pacer, dst, tiles, r, r1, r2, m, z=0):
    for j in range(0, m, 16):
      w11, w12, w21, w22 = (_unpack(tiles[z + t, (lo + j) // 2:(lo + j) // 2 + 8, :]).astype(F32)
                            for lo in (r1, r2) for t in (0, 1))
      lhs = _strassen_lhs(pacer.anchor(w11), w12, w21, pacer.anchor(w22))
      for i, w in enumerate(lhs[:2] + lhs[4:]):
        dst[i, r + j:r + j + 16, :] = w
        if i % 2 == 0:
          yield [w[8:]]

  def product(pacer, sums, tiles, r, r1, r2, m, enc, z, bias=None):
    summed = lambda i, e: pacer.dot(sums[z + i, r:r + m, :], enc[z0 + e])
    plain = lambda t, lo, e: pacer.dot(tiles[z + t, lo // 2:(lo + m) // 2, :], enc[z0 + e])
    biased = lambda x, lo: x if bias is None else x + bias[z0, lo:lo + m, :]
    m3 = pacer.mark(plain(0, r1, 2))
    p1 = biased(plain(2, r1, 7), r1)
    p1 = summed(2, 4) + p1
    c1b = plain(4, r1, 9) + (p1 + m3)
    m4 = pacer.mark(plain(1, r2, 3))
    p2 = biased(plain(2, r2, 7), r2)
    p2 = summed(1, 1) + p2
    c2a = plain(3, r2, 8) + (p2 + m4)
    m1 = pacer.mark(summed(0, 0))
    c1a = summed(4, 6) + ((p1 + m4) + m1)
    c1a = plain(3, r1, 8) + c1a
    c2b = summed(3, 5) + ((p2 + m3) - m1)
    c2b = plain(4, r2, 9) + c2b
    return c1a, c1b, c2a, c2b

  def eight_heads(pacer, sums, tiles, chunk, enc, z):
    c = product(pacer, sums, tiles, G * chunk, 2 * G * chunk, 2 * G * chunk + G, G, enc, z)
    return jnp.concatenate([jnp.concatenate(c[i:i + 2], axis=1) for i in (0, 2)], axis=0)

  row = lax.broadcasted_iota(I32, (HP, TB), 0)
  own = (row < DH, row >= HP - DH)

  def norm1(p, dst, via_memory=True):
    return layernorm(lambda rows: x_v[rows, cols(p)].astype(F32), dst, via_memory)

  def prep_qkv(pacer, chunk):
    transpose_tiles(wqkv_t, wqkv_v, ((0, 256), (256, 256), (512, 256), (768, 128), (896, 256), (1152, 192))[chunk])
    _run(tile_sums(pacer, wqkv_s, wqkv_t, G * chunk, 2 * G * chunk, 2 * G * chunk + G, G))

  def qkv(pacer, p, enc, chunk, z=0):
    t = eight_heads(pacer, wqkv_s, wqkv_t, chunk, enc, z)
    if chunk < 2:
      t = t * QSCALE
    for j in range(8):
      h, w = 8 * (chunk % 2) + j, t[_window(j):_window(j) + HP]
      if chunk < 2:
        q_s[h, :, cols(p)] = _pack(jnp.where(own[j % 2], w, 0.0))
        for i in range(2):
          _store_cyclic(qc_s.at[h, 2 * p + i], w[:, 128 * i:128 * (i + 1)], j % 2)
      elif chunk < 4:
        k_s[h, _at(p * 128, 128, 128), :] = _pack(jnp.concatenate([w.astype(BF)] * 4, axis=0).T)
        if isinstance(p, int) and p == 0:
          for i in range(2):
            _store_cyclic(kc_s.at[h, i], w[:, 128 * i:128 * (i + 1)], j % 2)
      else:
        v_s[h, :, cols(p)] = _pack(jnp.where(own[j % 2], w, 1.0))

  def skew_keys(h):
    lane = lax.broadcasted_iota(I32, (DH, 128), 1) & 7
    for t, n in enumerate((128, NV - 128)):
      skew = kc_s[z0 + h, t, 0:DH, :]
      for r in range(1, 8):
        skew = jnp.where(lane == r, kc_s[z0 + h, t, r:r + DH, :], skew)
      skew_s[h, t * 128:t * 128 + n, :] = skew.T[:n]

  def spread_keys(h, dst):
    for d in range(DH):
      column = jnp.broadcast_to(skew_s[h][:, d:d + 1], (NV, 128))
      dst[0, d] = column.reshape(NV // 8, 8, 128)
      yield [column[-8:]]

  pacer = _Pacer(z0)
  wait(0)
  prep_qkv(pacer, 0)
  wait(1)
  _run(norm1(0, e1))
  wait(2)
  pacer.add(norm1(1, e2, False), 64, 28)
  qkv(pacer, 0, e1, 0, z0)
  pacer.finish()
  wait(3)
  pacer = _Pacer(z0)
  qkv(pacer, 1, e2, 0, z0)
  prep_qkv(pacer, 1)
  qkv(pacer, 0, e1, 1)
  wait(4)
  pacer = _Pacer(z0)
  qkv(pacer, 1, e2, 1, z0)
  prep_qkv(pacer, 4)
  qkv(pacer, 0, e1, 4)
  prep_qkv(pacer, 5)
  wait(5)
  pacer = _Pacer(z0)
  qkv(pacer, 1, e2, 4, z0)
  prep_qkv(pacer, 2)
  pacer.add(norm1(2, e0), 64, 124)
  qkv(pacer, 0, e1, 2)
  prep_qkv(pacer, 3)
  for p, chunk in ((1, 2), (0, 3), (0, 5), (1, 3), (1, 5)):
    qkv(pacer, p, (e1, e2)[p], chunk)
  pacer.finish()
  wait(6)

  @pl.loop(1, NB // 2)
  def _(i):
    pacer = _Pacer(z0)
    for n in range(5):
      skew_keys((i - 1) * 5 + n + 1)
    for k in range(2):
      pacer.add(norm1(jnp.minimum(2 * i + k + 1, NB - 1), (e1, e0)[k]), 64, 124)
      for chunk in (4, 2, 0, 3, 1, 5):
        qkv(pacer, 2 * i + k, (e0, e1)[k], chunk, zs[k])
      pacer.finish()

  wait(7)

  def vpu_scores(h, table, done):
    for b in range(NB):
      for r in range(0, VPU_KEYS[b], 16):
        hq = h + zs[r // 16 % NB]
        for d in range(DH):
          k = lax.broadcast_in_dim(table[zs[b], d, r // 8:r // 8 + 2], (2, 2, 8, 128), (0, 2, 3))
          q = lax.broadcast_in_dim(qc_s[hq, 2 * b:2 * b + 2, d:d + 8, :], (2, 2, 8, 128), (1, 2, 3))
          acc = lax.add(acc, lax.mul(k, q)) if d else lax.mul(k, q)
          if d == DH - 1:
            done.append((b, r, jnp.concatenate([acc[:, t].reshape(16, 128) for t in range(2)], axis=1)))
          yield lambda slot, acc=acc: [acc[divmod((0, 2, 3, 1)[slot % 4], 2)]]

  def attend(pacer, h, blocks, carry, tables=None, prepare=None, filler=None):
    top, row_max = carry
    top, closed, done, held = ({} if top is None else {-1: top}), [], [], []
    first, last = row_max is None, blocks < NB
    if tables is not None:
      slots = sum((S - n) // 32 + 2 * NC for n in VPU_KEYS)
      pacer.add(vpu_scores(h, tables[0], done), sum(VPU_KEYS) // 16 * DH, slots + 3, lead=5, ramp=7)
      pacer.add(spread_keys(jnp.minimum(h + 1, H - 1), tables[1]), DH, slots)

    def paced(operand, shifts):
      return jnp.concatenate([pacer.tie(operand[i:i + 8], None if tables is None else shifts[i // 8])
                              for i in range(0, operand.shape[0], 8)], axis=0)

    def weigh(b, c):
      hb = h - 1 if b < 0 else h
      p = jnp.exp2(scores[b % 4][z0, c * KC:(c + 1) * KC, :] - row_max)
      v = v_s[hb, :, c * KC:(c + 1) * KC]
      v = jnp.concatenate([paced(v[:, :128], VALUE_SHIFT), v[:, 128:]], axis=1)
      acc = _dot(_unpack(v), p.astype(BF) if first else p)
      if c > 0:
        acc = acc + (held.pop() if held else acc_s[z0])
      if c == NC - 1:
        o_s[hb, :, cols(b % NB)] = acc
      else:
        held.append(acc)

    for b in range(blocks):
      if prepare is not None:
        prepare(b)
      cuts = _key_cuts(0 if tables is None else VPU_KEYS[b])
      if tables is not None and b == 0:
        cuts[1] -= 16
      if tables is not None and b == NB - 1:
        cuts[-2] += 16
      for c in range(NC):
        for j in range(0 if last else 2):
          lo, hi = cuts[2 * c + j], cuts[2 * c + j + 1]
          k = k_s[h, lo // 2:hi // 2, :]
          s = _dot(_unpack(k if j else paced(k, KEY_SHIFT))[:, :HP], _unpack(q_s[h, :, cols(b)]))
          scores[b % 4][0, lo:hi, :] = s
          pacer.passes += 4
          pacer.mark(s)
          part = jnp.max(s.reshape(-1, 8, TB), axis=0)
          top[b] = jnp.maximum(top[b], part) if b in top else part
        if filler is not None:
          filler(b, c)
        u, chunk = divmod((b - 1) * NC + c - LAG, NC)
        if not (first and u < 0 or last and u >= 0):
          if chunk == 0:
            row_max = jnp.max(top.pop(u), axis=0, keepdims=True)
            closed.append(u)
          weigh(u, chunk)
        if c == NC - 1 and (first or b == blocks - 1):
          pacer.finish()
        for u, r, s in done:
          assert u not in closed
          scores[u % 4][0, r:r + 16, :] = s
          top[u] = jnp.maximum(jnp.maximum(top[u], s[0:8]) if u in top else s[0:8], s[8:16])
        done.clear()
    if not last:
      acc_s[0] = held.pop()
      return top[NB - 1], row_max

  def w2_sums(pacer):
    for r in range(0, G, 16):
      for c in range(4):
        for i in range(7):
          def outer(r, c):
            return _strassen_lhs(*[w2t_v[r + dr:r + dr + 16, _at(zs[i] + 128 * c + dc, 128, 128)].astype(F32)
                                   for dr in (0, D // 2) for dc in (0, F // 2)])[i]

          if c < 3:
            w11, w12, w21, w22 = (outer(r + dr, c + dc) for dr in (0, G) for dc in (0, 3))
            words = [_pack(w) for w in _strassen_lhs(pacer.anchor(w11), w12, w21, pacer.anchor(w22))]
          else:
            words = [_pack(outer(r + dr, 6)) for dr in (0, G)]
          for j, w in enumerate(words):
            w2_s[i, 3 * j + c if c < 3 else 21 + j, r // 2:r // 2 + 8, :] = w
          yield words[:3]
          yield words[3:]

  def bias_column(dst, src):
    b = src[...].astype(F32).reshape(1, -1)
    for lo in range(0, b.shape[1], 256):
      part = b[:, lo:lo + 256]
      dst[0, lo:lo + part.shape[1], :] = jnp.broadcast_to(part, (128, part.shape[1])).T

  def prepare(b):
    slots = 8 * NC + 2 * (LAG * (b > 1) + (NC - LAG) * (b > 0))
    if b == 0:
      transpose_tiles(wo_t, wo_v, (0, 256), (256, 192))
      transpose_tiles(w1_t, w1_v, *[(c, 256) for c in range(0, F, 256)])
      bias_column(b2_c, b2_v)
      bias_column(b1_c, b1_v)
      _run(spread_keys(z0 + 1, kb1))
    if b < 6:
      n = 392 * (b + 1) // 6 - 392 * b // 6
      pacer.add(_take(w2_task, n) if b < 5 else w2_task, n, slots)
    else:
      k = b - 6
      pacer.add(_chain(tile_sums(pacer, wo_s, wo_t, G * k, 2 * G * k, 2 * G * k + G, G, z0),
                       tile_sums(pacer, w1_s, w1_t, D * k, D * k, F // 2 + D * k, D, z0)), 105, slots)

  def head(h, odd, carry):
    return attend(_Pacer(z0), h, NB, carry, (kb1, kb0) if odd else (kb0, kb1))

  pacer = _Pacer(z0)
  w2_task = w2_sums(pacer)
  carry = attend(pacer, z0, NB, (None, None), prepare=prepare)
  carry = lax.fori_loop(0, H // 2, lambda i, c: head(2 * i + 1, True, lax.cond(
      i > 0, functools.partial(head, 2 * i, False), lambda c: c, c)), carry)

  low = lax.broadcasted_iota(I32, (8, TB), 0) < HP - DH

  def gather_heads(p, dst, pacer=None):
    scales = []
    for h in range(0, H, 2):
      total = jnp.where(low, o_s[z0 + h + 1, 0:8, cols(p)], o_s[z0 + h, 24:32, cols(p)])
      if pacer is not None:
        total = jnp.concatenate([pacer.anchor(total[:, c:c + 128], 8) for c in (0, 128)], axis=1)
      scales.append(1.0 / total)
      yield [scales[-1], scales[-1][:, 128:]]

    def load(r):
      pair, j = divmod(r // 8, 7)
      even = o_s[z0 + 2 * pair, 8 * j:8 * j + 8, cols(p)] * scales[pair][7:8] if j <= 3 else None
      odd = o_s[z0 + 2 * pair + 1, 8 * j - 24:8 * j - 16, cols(p)] * scales[pair][0:1] if j >= 3 else None
      return jnp.where(low, even, odd) if j == 3 else (even if j < 3 else odd)

    yield from encode(lambda r: jnp.concatenate([load(r), load(r + 8)], axis=0), dst)

  def project(pacer, p, chunk):
    rows = pl.ds(2 * G * chunk, 2 * G)
    h = x_v[rows, cols(p)].astype(F32) + eight_heads(pacer, wo_s, wo_t, chunk, (e1, e2)[p % 2], zs[p])
    h_s[p, rows, :] = h
    if p == 0:
      h0_s[0, rows, :] = h

  def norm2(src, p, dst):
    return layernorm(lambda rows: src[p, rows, :], dst)

  pacer = _Pacer(z0)
  _run(gather_heads(0, e1))
  pacer.add(gather_heads(1, e2), 44, 52)
  attend(pacer, H, 2, carry, filler=lambda b, c: project(pacer, 0, c // 7) if b == 0 and c in (4, 7) else None)
  norm_task = norm2(h0_s, 0, e0)
  for p in range(1, NB):
    if p > 1:
      n = (6, 8, 8, 8, 8, 26)[p - 2]
      pacer.add(_take(norm_task, n) if p + 1 < NB else norm_task, n, 46)
    if p + 1 < NB:
      pacer.add(gather_heads(p + 1, (e2, e1)[p % 2], pacer), 44, 20)
    for chunk in range(2):
      project(pacer, p, chunk)
    pacer.finish()

  def out_copy(p, r, t):
    rows = pl.ds(r * (D // 2), D // 2)
    return pltpu.make_async_copy(out_v.at[p, rows, pl.ds(t * 128, 128)],
                                 out_hbm.at[rows, _at(p * TB + t * 128, 128, 128)], out_sem)

  @pl.loop(0, NB // 2)
  def ffn(step):
    p = 2 * step
    pacer = _Pacer(z0)
    for k in range(2):
      pacer.add(norm2(h_s, jnp.minimum(p + k + 1, NB - 1), (e1, e0)[k]), 64, 170)
      for c in range(7):
        pre = product(pacer, w1_s, w1_t, 128 * c, 128 * c, F // 2 + 128 * c, 128, (e0, e1)[k], zs[k], b1_c)
        a1, b1, a2, b2 = (r * r for r in (jnp.maximum(x, 0.0) for x in pre))
        for i, x in enumerate(_strassen_rhs(a1, a2, b1, b2)):
          (act_s, rest_s)[c // 6][i, k, c % 6] = x
      pacer.finish()

    def outer(i, bias=None):
      def inner(j):
        z = zs[(0, 1, 1, 2, 2, 3, 3)[j]]
        x = _strassen_rhs(*[act_s[z + i, k, c:c + 3].reshape(384, 128) for k in (0, 1) for c in (0, 3)])[j]
        return pacer.dot(jnp.concatenate([w2_s[z0 + i, 3 * j + c, :G // 2, :] for c in range(3)], axis=1), x)

      rest = lambda r, k: pacer.dot(w2_s[zs[k] + i, 21 + r, :G // 2, :], rest_s[zs[r] + i, k, 0])
      n2 = inner(1) if bias is None else inner(1) + bias[G:]
      n4 = inner(3)
      n5 = inner(4) if bias is None else inner(4) + bias[:G]
      n3 = inner(2)
      c21 = rest(1, 0) + (n2 + n4)
      c12 = rest(0, 1) + (n5 + n3)
      n1 = inner(0)
      c11 = inner(6) + ((n5 + n4) + n1)
      c11 = rest(0, 0) + c11
      c22 = inner(5) + ((n2 + n3) - n1)
      c22 = rest(1, 1) + c22
      return jnp.concatenate([c11, c21, c12, c22], axis=0).reshape(2, D // 2, 128)

    part = lambda r, t: (pl.ds(r * (D // 2), D // 2), pl.ds(t * 128, 128))
    resid = lambda r, t: h_s[(pl.ds(p, 2), *part(r, t))]

    def emit(r, t, x):
      for k in range(2):
        out_v[(p + k, *part(r, t))] = x[k].astype(BF)
        out_copy(p + k, r, t).start()

    m2 = outer(1, b2_c[z0, D // 2:, :])
    m4 = outer(3)
    emit(1, 0, resid(1, 0) + m2 + m4)
    m5 = outer(4, b2_c[z0, :D // 2, :])
    m3 = outer(2)
    emit(0, 1, resid(0, 1) + m5 + m3)
    m1 = outer(0)
    emit(0, 0, outer(6) + (resid(0, 0) + m5 + m4 + m1))
    emit(1, 1, outer(5) + (resid(1, 1) + m2 + m3 - m1))

  for p in range(NB):
    for r in range(2):
      for t in range(2):
        out_copy(p, r, t).wait()


@jax.jit
def pallas_sequential_preLN__softmax_full_mha__dense_activation_squared_relu__prompt_kernel(
    A_x: jax.Array,
    A_wqkv: jax.Array,
    A_wo: jax.Array,
    B_x: jax.Array,
    B_w1: jax.Array,
    B_b1: jax.Array,
    B_w2: jax.Array,
    B_b2: jax.Array,
):
  del B_x
  hbm = pl.BlockSpec(memory_space=pltpu.HBM)
  vmem = pltpu.VMEM
  out_t = pl.pallas_call(
      _block_kernel,
      out_shape=jax.ShapeDtypeStruct((D, S), BF),
      in_specs=[hbm] * 7,
      out_specs=hbm,
      scratch_shapes=[
          vmem((D, S), BF), vmem((D, 3 * D), BF), vmem((D, D), BF), vmem((D, F), BF), vmem((D, F), BF),
          vmem((5, 3 * D // 2, 128), I32), vmem((5, D // 2, 128), I32), vmem((5, F // 2, 128), I32),
          vmem((5, 3 * D // 2, 128), F32), vmem((5, D // 2, 128), F32), vmem((5, F // 2, 128), F32),
          vmem((7, 23, 64, 128), I32), vmem((1, F, 128), F32), vmem((1, D, 128), F32),
          vmem((H, HP // 2, S), I32), vmem((H, S // 2, 128), I32), vmem((H, HP // 2, S), I32),
          vmem((H, HP, S), F32), vmem((NB, D, TB), F32), vmem((NB, D, TB), BF),
          vmem((H, S // 128, 48, 128), F32), vmem((H, 2, 40, 128), F32), vmem((H, NV, DH), F32),
          vmem((1, DH, NV // 8, 8, 128), F32), vmem((1, DH, NV // 8, 8, 128), F32), vmem((1, HP, TB), F32),
          *[vmem((10, 128, 128), F32)] * 3,
          vmem((7, 2, 6, 128, 128), F32), vmem((7, 2, 1, 128, 128), F32), vmem((1, D, TB), F32),
          *[vmem((1, S, TB), F32)] * 4,
          vmem((F,), BF), vmem((D,), BF),
          pltpu.SemaphoreType.DMA((8,)), pltpu.SemaphoreType.DMA(()), pltpu.SMEM((NB,), I32),
      ],
      compiler_params=pltpu.CompilerParams(vmem_limit_bytes=100 * 1024 * 1024),
  )(A_x.reshape(S, D).T, A_wqkv, A_wo, B_w1, B_b1, B_w2.T, B_b2)
  return out_t.T.reshape(1, S, D)
```

```python
import functools
import math

import jax
import jax.numpy as jnp
from jax import lax
import jax.experimental.pallas as pl
import jax.experimental.pallas.tpu as pltpu

S, D, H, DH, F = 2048, 448, 16, 28, 1792
TB = 256
NB = S // TB
KC = 256
NC = S // KC
G = 4 * DH
HP = 32
NV = 192
VPU_KEYS = (192, 192, 192, 192, 192, 160, 192, 160)
LAG = 2
KEY_SHIFT = (3, 3, 3, 2, 2, 4, 7, 5, 5)
VALUE_SHIFT = (3, 4)
EPS = 1e-5
QSCALE = DH ** -0.5 * math.log2(math.e)
BF, F32, I32 = jnp.bfloat16, jnp.float32, jnp.int32


def _dot(a, b):
  return lax.dot_general(a, b, (((1,), (0,)), ((), ())), preferred_element_type=F32)


def _pack(x):
  return pltpu.bitcast(x.astype(BF), I32)


def _unpack(x):
  return pltpu.bitcast(x, BF)


def _at(start, size, align):
  return pl.ds(start if isinstance(start, int) else pl.multiple_of(start, align), size)


def _fold(x):
  return functools.reduce(jnp.add, [x[i:i + 8] for i in range(0, x.shape[0], 8)])


def _chain(*tasks):
  for task in tasks:
    yield from task


def _take(task, n):
  for _, piece in zip(range(n), task):
    yield piece


def _run(task):
  for _ in task:
    pass


def _window(h):
  return DH * h - (HP - DH) * (h % 2)


def _store_cyclic(dst, w, odd):
  if odd:
    dst[4:36, :] = w
    dst[0:8, :] = w[24:32]
  else:
    dst[0:32, :] = w
    dst[28:36, :] = w[0:8]


def _strassen_lhs(w11, w12, w21, w22):
  return [w11 + w22, w21 + w22, w11, w22, w11 + w12, w21 - w11, w12 - w22]


def _strassen_rhs(a1, a2, b1, b2):
  return [a1 - b2, a1, b1 - b2, a2 - a1, b2, b1 - a1, a2 - b2]


def _key_cuts(first):
  sizes = [(S - first) // 32 // NC] * NC
  for j in range((S - first) // 32 % NC):
    sizes[(2 * j + 2 * j // NC) % NC] += 1
  cuts = [first]
  for n in sizes:
    cuts += [cuts[-1] + 16 * n, cuts[-1] + 32 * n]
  return cuts


class _Pacer:
  def __init__(self, zero):
    self.never = lax.broadcasted_iota(I32, (8, 128), 0) < zero
    self.tasks, self.passes, self.results = [], 0, []

  def add(self, task, pieces, slots, lead=0, ramp=0):
    self.tasks.append(dict(task=task, pieces=pieces, slots=slots, slot=0, issued=-lead, ramp=ramp))

  def tie(self, vreg, shift=None):
    for t in self.tasks:
      t["slot"] += 1
      goal = t["pieces"] * t["slot"] // t["slots"] + (shift or 0) - max(0, t["ramp"] - t["slot"])
      values = [next(t["task"], []) for _ in range(t["issued"], goal)]
      t["issued"] = max(t["issued"], goal)
      if shift is not None:
        values = [v(t["slot"]) if callable(v) else v for v in values[-1:]]
        shift = 0
      for x in sum(values, []):
        x = x[0:8, 0:128]
        vreg = lax.select(self.never, x if x.dtype == vreg.dtype else pltpu.bitcast(x, vreg.dtype), vreg)
    return vreg

  def dot(self, lhs, rhs):
    step = 8 if lhs.dtype == I32 else 16
    tiles = []
    for c in range(0, lhs.shape[1], 128):
      tile = lhs[:, c:c + 128]
      if self.tasks and self.passes % 4 == 0:
        tile = jnp.concatenate([tile[i:i + 8] if i % step else self.tie(tile[i:i + 8])
                                for i in range(0, tile.shape[0], 8)], axis=0)
      self.passes += 1
      tiles.append(tile)
    lhs = jnp.concatenate(tiles, axis=1)
    return _dot(_unpack(lhs) if lhs.dtype == I32 else lhs, rhs)

  def mark(self, x):
    self.results.append((self.passes, x))
    return x

  def anchor(self, x, back=16):
    old = [r for n, r in self.results if n <= self.passes - back]
    if not old:
      return x
    return jnp.concatenate([lax.select(self.never, old[-1][0:8, 0:128], x[i:i + 8])
                            for i in range(0, x.shape[0], 8)], axis=0)

  def finish(self):
    for t in self.tasks:
      _run(t["task"])
    self.tasks = []


def _block_kernel(x_hbm, wqkv_hbm, wo_hbm, w1_hbm, b1_hbm, w2t_hbm, b2_hbm, out_hbm,
                  x_v, wqkv_v, wo_v, w1_v, w2t_v, wqkv_t, wo_t, w1_t, wqkv_s, wo_s, w1_s, w2_s, b1_c, b2_c,
                  q_s, k_s, v_s, o_s, h_s, out_v, qc_s, kc_s, skew_s, kb_s, acc_s, e0, e1, e2,
                  act_s, rest_s, h0_s, s0, s1, s2, s3, b1_v, b2_v, in_sem, out_sem, zero_s):
  scores = (s0, s1, s2, s3)
  cols = lambda p: _at(p * TB, TB, TB)

  xs = lambda lo, hi: (x_hbm.at[:, lo * TB:hi * TB], x_v.at[:, lo * TB:hi * TB])
  ws = lambda lo, hi: (wqkv_hbm.at[:, lo:hi], wqkv_v.at[:, lo:hi])
  stages = [[ws(0, 256)], [xs(0, 1)], [xs(1, 2)], [ws(256, 512)], [ws(896, 3 * D)], [ws(512, 896), xs(2, 3)],
            [xs(3, NB)], [(wo_hbm, wo_v), (b1_hbm, b1_v), (b2_hbm, b2_v), (w2t_hbm, w2t_v), (w1_hbm, w1_v)]]
  stages = [[pltpu.make_async_copy(src, dst, in_sem.at[i]) for src, dst in stage]
            for i, stage in enumerate(stages)]
  for copy in sum(stages, []):
    copy.start()

  def wait(i):
    for copy in stages[i]:
      copy.wait()

  @pl.loop(0, NB)
  def _(i):
    zero_s[i] = 0

  zs = [zero_s[i] for i in range(NB)]
  z0 = zs[0]

  def encode(load, dst, via_memory=False):
    def put(i, r, x):
      dst[i, r:r + 16, :] = x
      return [x[8:]]

    for r in range(0, 128, 16):
      x1, x2 = load(r), load(128 + r)
      e = [put(i, r, x) for i, x in enumerate(_strassen_rhs(x1[:, :128], x2[:, :128], x1[:, 128:], x2[:, 128:]))]
      yield from ([], [], [dst[z0 + 6, r:r + 8, :]]) if via_memory else (e[0], e[2] + e[5], e[3] + e[6])
    for r in range(0, 64, 16):
      u, v, w = load(256 + r), load(320 + r), load(384 + r)
      au, bv = u[:, :128].astype(BF).astype(F32), v[:, 128:].astype(BF).astype(F32)
      halves = ((au, bv), (v[:, :128] - bv, w[:, :128]), (u[:, 128:] - au, w[:, 128:]))
      e = [put(7 + i, r, lo) + put(7 + i, 64 + r, hi) for i, (lo, hi) in enumerate(halves)]
      yield from ([], [], [dst[z0 + 9, r:r + 8, :]]) if via_memory else e

  def layernorm(load, dst, via_memory=False):
    for r in range(0, D, 32):
      part = _fold(load(_at(zs[1] + r, 32, 16)))
      acc = acc + part if r else part
      yield [acc, acc[:, 128:]]
    mean = jnp.sum(acc, axis=0, keepdims=True) * (1.0 / D)
    for r in range(0, D, 32):
      centred = load(_at(zs[2] + r, 32, 16)) - mean
      part = _fold(centred * centred)
      acc = acc + part if r else part
      yield [acc, acc[:, 128:]]
    rstd = lax.rsqrt(jnp.sum(acc, axis=0, keepdims=True) * (1.0 / D) + EPS)
    yield from encode(lambda r: (load(_at(zs[3] + r, 16, 16)) - mean) * rstd, dst, via_memory)

  def transpose_tiles(dst, src, *spans):
    u, v, w = 256, 320, 384
    for t, parts in ((0, [(0, 128)]), (1, [(128, 128)]), (2, [(u, 128)]), (4, [(u, 64), (w, 64)]), (3, [(v, 128)])):
      for c, n in spans:
        dst[t, c // 2:(c + n) // 2, :] = _pack(jnp.concatenate([src[r:r + k, c:c + n] for r, k in parts], axis=0).T)

  def tile_sums(pacer, dst, tiles, r, r1, r2, m, z=0):
    for j in range(0, m, 16):
      w11, w12, w21, w22 = (_unpack(tiles[z + t, (lo + j) // 2:(lo + j) // 2 + 8, :]).astype(F32)
                            for lo in (r1, r2) for t in (0, 1))
      lhs = _strassen_lhs(pacer.anchor(w11), w12, w21, pacer.anchor(w22))
      for i, w in enumerate(lhs[:2] + lhs[4:]):
        dst[i, r + j:r + j + 16, :] = w
        if i % 2 == 0:
          yield [w[8:]]

  def product(pacer, sums, tiles, r, r1, r2, m, enc, z, bias=None):
    summed = lambda i, e: pacer.dot(sums[z + i, r:r + m, :], enc[z0 + e])
    plain = lambda t, lo, e: pacer.dot(tiles[z + t, lo // 2:(lo + m) // 2, :], enc[z0 + e])
    biased = lambda x, lo: x if bias is None else x + bias[z0, lo:lo + m, :]
    m3 = pacer.mark(plain(0, r1, 2))
    p1 = biased(plain(2, r1, 7), r1)
    p1 = summed(2, 4) + p1
    c1b = plain(4, r1, 9) + (p1 + m3)
    m4 = pacer.mark(plain(1, r2, 3))
    p2 = biased(plain(2, r2, 7), r2)
    p2 = summed(1, 1) + p2
    c2a = plain(3, r2, 8) + (p2 + m4)
    m1 = pacer.mark(summed(0, 0))
    c1a = summed(4, 6) + ((p1 + m4) + m1)
    c1a = plain(3, r1, 8) + c1a
    c2b = summed(3, 5) + ((p2 + m3) - m1)
    c2b = plain(4, r2, 9) + c2b
    return c1a, c1b, c2a, c2b

  def eight_heads(pacer, sums, tiles, chunk, enc, z):
    c = product(pacer, sums, tiles, G * chunk, 2 * G * chunk, 2 * G * chunk + G, G, enc, z)
    return jnp.concatenate([jnp.concatenate(c[i:i + 2], axis=1) for i in (0, 2)], axis=0)

  row = lax.broadcasted_iota(I32, (HP, TB), 0)
  own = (row < DH, row >= HP - DH)

  def norm1(p, dst, via_memory=True):
    return layernorm(lambda rows: x_v[rows, cols(p)].astype(F32), dst, via_memory)

  def prep_qkv(pacer, chunk):
    transpose_tiles(wqkv_t, wqkv_v, ((0, 256), (256, 256), (512, 256), (768, 128), (896, 256), (1152, 192))[chunk])
    _run(tile_sums(pacer, wqkv_s, wqkv_t, G * chunk, 2 * G * chunk, 2 * G * chunk + G, G))

  def qkv(pacer, p, enc, chunk, z=0):
    t = eight_heads(pacer, wqkv_s, wqkv_t, chunk, enc, z)
    if chunk < 2:
      t = t * QSCALE
    for j in range(8):
      h, w = 8 * (chunk % 2) + j, t[_window(j):_window(j) + HP]
      if chunk < 2:
        q_s[h, :, cols(p)] = _pack(jnp.where(own[j % 2], w, 0.0))
        for i in range(2):
          _store_cyclic(qc_s.at[h, 2 * p + i], w[:, 128 * i:128 * (i + 1)], j % 2)
      elif chunk < 4:
        k_s[h, _at(p * 128, 128, 128), :] = _pack(jnp.concatenate([w.astype(BF)] * 4, axis=0).T)
        if isinstance(p, int) and p == 0:
          for i in range(2):
            _store_cyclic(kc_s.at[h, i], w[:, 128 * i:128 * (i + 1)], j % 2)
      else:
        v_s[h, :, cols(p)] = _pack(jnp.where(own[j % 2], w, 1.0))

  def skew_keys(h):
    lane = lax.broadcasted_iota(I32, (DH, 128), 1) & 7
    for t, n in enumerate((128, NV - 128)):
      skew = kc_s[z0 + h, t, 0:DH, :]
      for r in range(1, 8):
        skew = jnp.where(lane == r, kc_s[z0 + h, t, r:r + DH, :], skew)
      skew_s[h, t * 128:t * 128 + n, :] = skew.T[:n]

  def spread_keys(h, dst, slot):
    for d in range(DH):
      column = jnp.broadcast_to(skew_s[h][:, d:d + 1], (NV, 128))
      dst[slot, d] = column.reshape(NV // 8, 8, 128)
      yield [column[-8:]]

  pacer = _Pacer(z0)
  wait(0)
  prep_qkv(pacer, 0)
  wait(1)
  _run(norm1(0, e1))
  wait(2)
  pacer.add(norm1(1, e2, False), 64, 28)
  qkv(pacer, 0, e1, 0, z0)
  pacer.finish()
  wait(3)
  pacer = _Pacer(z0)
  qkv(pacer, 1, e2, 0, z0)
  prep_qkv(pacer, 1)
  qkv(pacer, 0, e1, 1)
  wait(4)
  pacer = _Pacer(z0)
  qkv(pacer, 1, e2, 1, z0)
  prep_qkv(pacer, 4)
  qkv(pacer, 0, e1, 4)
  prep_qkv(pacer, 5)
  wait(5)
  pacer = _Pacer(z0)
  qkv(pacer, 1, e2, 4, z0)
  prep_qkv(pacer, 2)
  pacer.add(norm1(2, e0), 64, 110)
  qkv(pacer, 0, e1, 2)
  prep_qkv(pacer, 3)
  for p, chunk in ((1, 2), (0, 3), (0, 5), (1, 3), (1, 5)):
    qkv(pacer, p, (e1, e2)[p], chunk)
  pacer.finish()
  wait(6)
  pacer = _Pacer(z0)
  for p in range(2, NB):
    if p % 2 == 0:
      for h in range(5 * (p // 2) - 4, 5 * (p // 2) + 1):
        skew_keys(h)
    if p + 1 < NB:
      pacer.add(norm1(p + 1, (e1, e0)[p % 2]), 64, 124)
    for chunk in (0, 2, 4, 3, 1, 5):
      qkv(pacer, p, (e0, e1)[p % 2], chunk, zs[p])
    pacer.finish()
  wait(7)

  def vpu_scores(h, tables, done):
    for b in range(NB):
      for r in range(0, VPU_KEYS[b], 16):
        hq = h + zs[r // 16 % NB]
        for d in range(DH):
          k = lax.broadcast_in_dim(tables[0, d, r // 8:r // 8 + 2], (2, 2, 8, 128), (0, 2, 3))
          q = lax.broadcast_in_dim(qc_s[hq, 2 * b:2 * b + 2, d:d + 8, :], (2, 2, 8, 128), (1, 2, 3))
          acc = lax.add(acc, lax.mul(k, q)) if d else lax.mul(k, q)
          if d == DH - 1:
            done.append((b, r, jnp.concatenate([acc[:, t].reshape(16, 128) for t in range(2)], axis=1)))
          yield lambda slot, acc=acc: [acc[divmod((0, 2, 3, 1)[slot % 4], 2)]]

  def attend(pacer, h, blocks, carry, tables=None, prepare=None, filler=None):
    top, row_max = carry
    top, closed, done, held = ({} if top is None else {-1: top}), [], [], []
    first, last = row_max is None, blocks < NB
    if tables is not None:
      slots = sum((S - n) // 32 + 2 * NC for n in VPU_KEYS)
      pacer.add(vpu_scores(h, tables, done), sum(VPU_KEYS) // 16 * DH, slots + 3, lead=5, ramp=8)
      pacer.add(spread_keys(jnp.minimum(h + 1, H - 1), tables, 1), DH, slots)

    def paced(operand, shifts):
      return jnp.concatenate([pacer.tie(operand[i:i + 8], None if tables is None else shifts[i // 8])
                              for i in range(0, operand.shape[0], 8)], axis=0)

    def weigh(b, c):
      hb = h - 1 if b < 0 else h
      p = jnp.exp2(scores[b % 4][z0, c * KC:(c + 1) * KC, :] - row_max)
      v = v_s[hb, :, c * KC:(c + 1) * KC]
      v = jnp.concatenate([paced(v[:, :128], VALUE_SHIFT), v[:, 128:]], axis=1)
      acc = _dot(_unpack(v), p.astype(BF) if first else p)
      if c > 0:
        acc = acc + (held.pop() if held else acc_s[z0])
      if c == NC - 1:
        o_s[hb, :, cols(b % NB)] = acc
      else:
        held.append(acc)

    for b in range(blocks):
      if prepare is not None:
        prepare(b)
      cuts = _key_cuts(0 if tables is None else VPU_KEYS[b])
      if tables is not None and b == 0:
        cuts[1] -= 16
      if tables is not None and b == NB - 1:
        cuts[-2] += 16
      for c in range(NC):
        for j in range(0 if last else 2):
          lo, hi = cuts[2 * c + j], cuts[2 * c + j + 1]
          k = k_s[h, lo // 2:hi // 2, :]
          s = _dot(_unpack(k if j else paced(k, KEY_SHIFT))[:, :HP], _unpack(q_s[h, :, cols(b)]))
          scores[b % 4][0, lo:hi, :] = s
          pacer.passes += 4
          pacer.mark(s)
          part = jnp.max(s.reshape(-1, 8, TB), axis=0)
          top[b] = jnp.maximum(top[b], part) if b in top else part
        if filler is not None:
          filler(b, c)
        u, chunk = divmod((b - 1) * NC + c - LAG, NC)
        if not (first and u < 0 or last and u >= 0):
          if chunk == 0:
            row_max = jnp.max(top.pop(u), axis=0, keepdims=True)
            closed.append(u)
          weigh(u, chunk)
        if c == NC - 1 and (first or b == blocks - 1):
          pacer.finish()
        for u, r, s in done:
          assert u not in closed
          scores[u % 4][0, r:r + 16, :] = s
          top[u] = jnp.maximum(jnp.maximum(top[u], s[0:8]) if u in top else s[0:8], s[8:16])
        done.clear()
    if not last:
      acc_s[0] = held.pop()
      return top[NB - 1], row_max

  def w2_sums(pacer):
    for r in range(0, G, 16):
      for c in range(4):
        for i in range(7):
          def outer(r, c):
            return _strassen_lhs(*[w2t_v[r + dr:r + dr + 16, _at(zs[i] + 128 * c + dc, 128, 128)].astype(F32)
                                   for dr in (0, D // 2) for dc in (0, F // 2)])[i]

          if c < 3:
            w11, w12, w21, w22 = (outer(r + dr, c + dc) for dr in (0, G) for dc in (0, 3))
            words = [_pack(w) for w in _strassen_lhs(pacer.anchor(w11), w12, w21, pacer.anchor(w22))]
          else:
            words = [_pack(outer(r + dr, 6)) for dr in (0, G)]
          for j, w in enumerate(words):
            w2_s[i, 3 * j + c if c < 3 else 21 + j, r // 2:r // 2 + 8, :] = w
          yield words[:3]
          yield words[3:]

  def bias_column(dst, src):
    b = src[...].astype(F32).reshape(1, -1)
    for lo in range(0, b.shape[1], 256):
      part = b[:, lo:lo + 256]
      dst[0, lo:lo + part.shape[1], :] = jnp.broadcast_to(part, (128, part.shape[1])).T

  def prepare(b):
    slots = 8 * NC + 2 * (LAG * (b > 1) + (NC - LAG) * (b > 0))
    if b == 0:
      transpose_tiles(wo_t, wo_v, (0, 256), (256, 192))
      transpose_tiles(w1_t, w1_v, *[(c, 256) for c in range(0, F, 256)])
      bias_column(b2_c, b2_v)
      bias_column(b1_c, b1_v)
      _run(spread_keys(z0 + 1, kb_s, 0))
    if b < 6:
      n = 392 * (b + 1) // 6 - 392 * b // 6
      pacer.add(_take(w2_task, n) if b < 5 else w2_task, n, slots)
    else:
      k = b - 6
      pacer.add(_chain(tile_sums(pacer, wo_s, wo_t, G * k, 2 * G * k, 2 * G * k + G, G, z0),
                       tile_sums(pacer, w1_s, w1_t, D * k, D * k, F // 2 + D * k, D, z0)), 105, slots)

  pacer = _Pacer(z0)
  w2_task = w2_sums(pacer)
  carry = attend(pacer, z0, NB, (None, None), prepare=prepare)
  carry = lax.fori_loop(1, H, lambda h, c: attend(_Pacer(z0), h, NB, c, kb_s.at[pl.ds(h - 1, 2)]), carry)

  low = lax.broadcasted_iota(I32, (8, TB), 0) < HP - DH

  def gather_heads(p, dst, pacer=None):
    scales = []
    for h in range(0, H, 2):
      total = jnp.where(low, o_s[z0 + h + 1, 0:8, cols(p)], o_s[z0 + h, 24:32, cols(p)])
      if pacer is not None:
        total = jnp.concatenate([pacer.anchor(total[:, c:c + 128], 6) for c in (0, 128)], axis=1)
      scales.append(1.0 / total)
      yield [scales[-1], scales[-1][:, 128:]]

    def load(r):
      pair, j = divmod(r // 8, 7)
      even = o_s[z0 + 2 * pair, 8 * j:8 * j + 8, cols(p)] * scales[pair][7:8] if j <= 3 else None
      odd = o_s[z0 + 2 * pair + 1, 8 * j - 24:8 * j - 16, cols(p)] * scales[pair][0:1] if j >= 3 else None
      return jnp.where(low, even, odd) if j == 3 else (even if j < 3 else odd)

    yield from encode(lambda r: jnp.concatenate([load(r), load(r + 8)], axis=0), dst)

  def project(pacer, p, chunk):
    rows = pl.ds(2 * G * chunk, 2 * G)
    h = x_v[rows, cols(p)].astype(F32) + eight_heads(pacer, wo_s, wo_t, chunk, (e1, e2)[p % 2], zs[p])
    h_s[p, rows, :] = h
    if p == 0:
      h0_s[0, rows, :] = h

  def norm2(src, p, dst):
    return layernorm(lambda rows: src[p, rows, :], dst)

  pacer = _Pacer(z0)
  _run(gather_heads(0, e1))
  pacer.add(gather_heads(1, e2), 44, 52)
  pacer.add(iter([[kb_s[z0, 0, 0]]]), 1, 1)
  attend(pacer, H, 2, carry, filler=lambda b, c: project(pacer, 0, c // 7) if b == 0 and c in (4, 7) else None)
  norm_task = norm2(h0_s, 0, e0)
  for p in range(1, NB):
    if p > 1:
      n = (6, 8, 8, 8, 8, 26)[p - 2]
      pacer.add(_take(norm_task, n) if p + 1 < NB else norm_task, n, 46)
    if p + 1 < NB:
      pacer.add(gather_heads(p + 1, (e2, e1)[p % 2], pacer), 44, 20)
    for chunk in range(2):
      project(pacer, p, chunk)
    pacer.finish()

  def out_copy(p, r, t):
    rows = pl.ds(r * (D // 2), D // 2)
    return pltpu.make_async_copy(out_v.at[p, rows, pl.ds(t * 128, 128)],
                                 out_hbm.at[rows, _at(p * TB + t * 128, 128, 128)], out_sem)

  @pl.loop(0, NB // 2)
  def ffn(step):
    p = 2 * step
    pacer = _Pacer(z0)
    for k in range(2):
      pacer.add(norm2(h_s, jnp.minimum(p + k + 1, NB - 1), (e1, e0)[k]), 64, 170)
      for c in range(7):
        pre = product(pacer, w1_s, w1_t, 128 * c, 128 * c, F // 2 + 128 * c, 128, (e0, e1)[k], zs[k], b1_c)
        a1, b1, a2, b2 = (r * r for r in (jnp.maximum(x, 0.0) for x in pre))
        for i, x in enumerate(_strassen_rhs(a1, a2, b1, b2)):
          (act_s, rest_s)[c // 6][i, k, c % 6] = x
      pacer.finish()

    def outer(i, bias=None):
      def inner(j):
        z = zs[(0, 1, 1, 2, 2, 3, 3)[j]]
        x = _strassen_rhs(*[act_s[z + i, k, c:c + 3].reshape(384, 128) for k in (0, 1) for c in (0, 3)])[j]
        return pacer.dot(jnp.concatenate([w2_s[z0 + i, 3 * j + c, :G // 2, :] for c in range(3)], axis=1), x)

      rest = lambda r, k: pacer.dot(w2_s[zs[k] + i, 21 + r, :G // 2, :], rest_s[zs[r] + i, k, 0])
      n2 = inner(1) if bias is None else inner(1) + bias[G:]
      n4 = inner(3)
      n5 = inner(4) if bias is None else inner(4) + bias[:G]
      n3 = inner(2)
      c21 = rest(1, 0) + (n2 + n4)
      c12 = rest(0, 1) + (n5 + n3)
      n1 = inner(0)
      c11 = inner(6) + ((n5 + n4) + n1)
      c11 = rest(0, 0) + c11
      c22 = inner(5) + ((n2 + n3) - n1)
      c22 = rest(1, 1) + c22
      return jnp.concatenate([c11, c21, c12, c22], axis=0).reshape(2, D // 2, 128)

    part = lambda r, t: (pl.ds(r * (D // 2), D // 2), pl.ds(t * 128, 128))
    resid = lambda r, t: h_s[(pl.ds(p, 2), *part(r, t))]

    def emit(r, t, x):
      for k in range(2):
        out_v[(p + k, *part(r, t))] = x[k].astype(BF)
        out_copy(p + k, r, t).start()

    m2 = outer(1, b2_c[z0, D // 2:, :])
    m4 = outer(3)
    emit(1, 0, resid(1, 0) + m2 + m4)
    m5 = outer(4, b2_c[z0, :D // 2, :])
    m3 = outer(2)
    emit(0, 1, resid(0, 1) + m5 + m3)
    m1 = outer(0)
    emit(0, 0, outer(6) + (resid(0, 0) + m5 + m4 + m1))
    emit(1, 1, outer(5) + (resid(1, 1) + m2 + m3 - m1))

  for p in range(NB):
    for r in range(2):
      for t in range(2):
        out_copy(p, r, t).wait()


@jax.jit
def pallas_sequential_preLN__softmax_full_mha__dense_activation_squared_relu__prompt_kernel(
    A_x: jax.Array,
    A_wqkv: jax.Array,
    A_wo: jax.Array,
    B_x: jax.Array,
    B_w1: jax.Array,
    B_b1: jax.Array,
    B_w2: jax.Array,
    B_b2: jax.Array,
):
  del B_x
  hbm = pl.BlockSpec(memory_space=pltpu.HBM)
  vmem = pltpu.VMEM
  out_t = pl.pallas_call(
      _block_kernel,
      out_shape=jax.ShapeDtypeStruct((D, S), BF),
      in_specs=[hbm] * 7,
      out_specs=hbm,
      scratch_shapes=[
          vmem((D, S), BF), vmem((D, 3 * D), BF), vmem((D, D), BF), vmem((D, F), BF), vmem((D, F), BF),
          vmem((5, 3 * D // 2, 128), I32), vmem((5, D // 2, 128), I32), vmem((5, F // 2, 128), I32),
          vmem((5, 3 * D // 2, 128), F32), vmem((5, D // 2, 128), F32), vmem((5, F // 2, 128), F32),
          vmem((7, 23, 64, 128), I32), vmem((1, F, 128), F32), vmem((1, D, 128), F32),
          vmem((H, HP // 2, S), I32), vmem((H, S // 2, 128), I32), vmem((H, HP // 2, S), I32),
          vmem((H, HP, S), F32), vmem((NB, D, TB), F32), vmem((NB, D, TB), BF),
          vmem((H, S // 128, 48, 128), F32), vmem((H, 2, 40, 128), F32), vmem((H, NV, DH), F32),
          vmem((H, DH, NV // 8, 8, 128), F32), vmem((1, HP, TB), F32),
          *[vmem((10, 128, 128), F32)] * 3,
          vmem((7, 2, 6, 128, 128), F32), vmem((7, 2, 1, 128, 128), F32), vmem((1, D, TB), F32),
          *[vmem((1, S, TB), F32)] * 4,
          vmem((F,), BF), vmem((D,), BF),
          pltpu.SemaphoreType.DMA((8,)), pltpu.SemaphoreType.DMA(()), pltpu.SMEM((NB,), I32),
      ],
      compiler_params=pltpu.CompilerParams(vmem_limit_bytes=120 * 1024 * 1024),
  )(A_x.reshape(S, D).T, A_wqkv, A_wo, B_w1, B_b1, B_w2.T, B_b2)
  return out_t.T.reshape(1, S, D)
```
